```python
import os as _os
_os.environ.setdefault("JAX_PLATFORMS", "cpu")
import jax
import jax.numpy as jnp

def _softmax(x, axis=-1):
    return jax.nn.softmax(x, axis=axis)
def _gelu(x):
    return jax.nn.gelu(x, approximate=True)
def _silu(x):
    return jax.nn.silu(x)
def _sigmoid(x):
    return jax.nn.sigmoid(x)
def _layernorm(x, axis=-1, eps=1e-5):
    m = jnp.mean(x, axis=axis, keepdims=True)
    v = jnp.var(x, axis=axis, keepdims=True)
    return (x - m) / jnp.sqrt(v + eps)
def _scatter_add(tgt, idx, src, axis=0):
    return tgt.at[idx].add(src)
def _segment_sum(src, seg, n):
    return jax.ops.segment_sum(src, seg, n)
class _Rng:
    def __init__(self, key):
        self._k = key
    def _next(self):
        self._k, sub = jax.random.split(self._k)
        return sub
    def normal(self, shape):
        return jax.random.normal(self._next(), shape, dtype=jnp.bfloat16)
    def randint(self, lo, hi, shape):
        return jax.random.randint(self._next(), shape, lo, hi, dtype=jnp.int32)
    def uniform(self, shape, lo=0.0, hi=1.0):
        return jax.random.uniform(self._next(), shape, jnp.bfloat16, lo, hi)
    def permutation(self, n):
        return jax.random.permutation(self._next(), n)


kernel_name = 'sequential_preLN__mha_block__mixer_token_mlp__prompt'

def setup_inputs():
    _rng = _Rng(jax.random.key(int.from_bytes(__import__("os").urandom(4), "little")))
    _w = (lambda a: (lambda t: t.astype(jnp.bfloat16) if jnp.issubdtype(t.dtype, jnp.floating) else t)(jnp.asarray(a)))
    def _A_setup():
        B, S, D, H = 1, 2048, 448, 16
        return {
            "x": _w((lambda *s: _rng.normal(s) * 0.05)(B, S, D)),
            "wqkv": _w((lambda *s: _rng.normal(s) * 0.05)(D, 3 * D)),
            "wo": _w((lambda *s: _rng.normal(s) * 0.05)(D, D)),
        }
    _A_in = _A_setup()

    def _B_setup():
        B, S, D, F = 1, 2048, 448, 1792
        return {
            "x": _w((lambda *s: _rng.normal(s) * 0.05)(B, S, D)),
            "w1": _w((lambda *s: _rng.normal(s) * 0.2)(S, F) * (S ** -0.5)),
            "b1": _w((lambda *s: _rng.normal(s) * 0.2)(F) * 0.02),
            "w2": _w((lambda *s: _rng.normal(s) * 0.2)(F, S) * (F ** -0.5)),
            "b2": _w((lambda *s: _rng.normal(s) * 0.05)(S) * 0.02),
        }
    _B_in = _B_setup()

    return {
        "A_x": _A_in["x"],
        "A_wqkv": _A_in["wqkv"],
        "A_wo": _A_in["wo"],
        "B_x": _B_in["x"],
        "B_w1": _B_in["w1"],
        "B_b1": _B_in["b1"],
        "B_w2": _B_in["w2"],
        "B_b2": _B_in["b2"],
    }

def reference(A_x, A_wqkv, A_wo, B_x, B_w1, B_b1, B_w2, B_b2):
    def _A_ref(x, wqkv, wo):
        B, S, D = x.shape
        H = 16
        Dh = D // H
        qkv = (lambda x, *d: x.transpose(*d))((x @ wqkv).reshape(B, S, 3, H, Dh), 2, 0, 3, 1, 4)
        q, k, v = qkv[0], qkv[1], qkv[2]
        scores = jnp.einsum("bhqd,bhkd->bhqk", q, k) * (Dh ** -0.5)
        p = _softmax(scores, axis=-1)
        o = jnp.einsum("bhqk,bhkd->bhqd", p, v)
        return (lambda x, *d: x.transpose(*d))(o, 0, 2, 1, 3).reshape(B, S, D) @ wo

    def _B_ref(x, w1, b1, w2, b2):
        B, S, D = x.shape
        h = _layernorm(x, axis=-1)
        u = jnp.einsum("bsd,sf->bdf", h, w1) + b1
        u = _gelu(u)
        y = jnp.einsum("bdf,fs->bds", u, w2) + b2
        return (lambda x, *d: x.transpose(*d))(y, 0, 2, 1)

    x = A_x
    h = x + _A_ref(_layernorm(x, axis=-1), A_wqkv, A_wo)
    h2 = h + _B_ref(_layernorm(h, axis=-1), B_w1, B_b1, B_w2, B_b2)
    return h2
```

```python
import functools

import jax
import jax.numpy as jnp
import jax.experimental.pallas as pl
import jax.experimental.pallas.tpu as pltpu

S = 2048
D = 448
H = 16
DH = 28
F = 1792
HP = 32
G = 4
GW = 4 * DH
EPS = 1e-5
LOG2E = 1.4426950408889634
QSCALE = (DH ** -0.5) * LOG2E

T1 = 512
QT = 512
KC = 128
T3 = 512
FT = 256
T5 = 256

NT = (((1,), (1,)), ((), ()))
F32 = jnp.float32
BF16 = jnp.bfloat16


def _dot(a, b):
    return jnp.dot(a, b, preferred_element_type=F32)


def _dot_nt(a, b):
    return jax.lax.dot_general(a, b, NT, preferred_element_type=F32)


def _gelu_tanh(x):
    c = 0.7978845608028654
    return 0.5 * x * (1.0 + jnp.tanh(c * (x + 0.044715 * (x * x * x))))


def _kernel(x_hbm, wqkv_hbm, wo_hbm, w1_hbm, b1_hbm, w2_hbm, b2_hbm, out_hbm,
            x_s, wqkv_s, wo_s, w1_s, b1_s, w2_s, b2_s,
            wk_p, wqv_t, wo_t, rep_s,
            k_s, qt_s, vt_s, ot_s, ht_s, ln2_s, g_s, out_s,
            in_sems, out_sems):
    n1 = S // T1

    def x_copy(c):
        return pltpu.make_async_copy(x_hbm.at[pl.ds(c * T1, T1)],
                                     x_s.at[pl.ds(c * T1, T1)], in_sems.at[c])

    wqkv_copy = pltpu.make_async_copy(wqkv_hbm, wqkv_s, in_sems.at[n1])
    wo_copy = pltpu.make_async_copy(wo_hbm, wo_s, in_sems.at[n1 + 1])
    b1_copy = pltpu.make_async_copy(b1_hbm, b1_s, in_sems.at[n1 + 2])
    b2_copy = pltpu.make_async_copy(b2_hbm, b2_s, in_sems.at[n1 + 3])
    w1_copy = pltpu.make_async_copy(w1_hbm, w1_s, in_sems.at[n1 + 4])
    w2_copy = pltpu.make_async_copy(w2_hbm, w2_s, in_sems.at[n1 + 5])

    wqkv_copy.start()
    for c in range(n1):
        x_copy(c).start()
    wo_copy.start()
    b1_copy.start()
    b2_copy.start()

    wqkv_copy.wait()
    w1_copy.start()
    w2_copy.start()

    wk_p[...] = jnp.zeros(wk_p.shape, BF16)
    for g in range(G):
        wk_p[:, 128 * g:128 * g + GW] = wqkv_s[:, D + GW * g:D + GW * (g + 1)]
    wqv_t[0:D, :] = wqkv_s[:, 0:D].astype(F32).T.astype(BF16)
    wvt = wqkv_s[:, 2 * D:3 * D].astype(F32).T
    rep_s[...] = jnp.zeros(rep_s.shape, F32)
    for h in range(H):
        rep_s[HP * h:HP * h + DH, :] = wvt[DH * h:DH * (h + 1), :]
    wqv_t[D:D + H * HP, :] = rep_s[...].astype(BF16)

    vrow = jax.lax.broadcasted_iota(jnp.int32, (H * HP, T1), 0)
    ones_row = (vrow % HP) == DH
    for c in range(n1):
        x_copy(c).wait()
        xf = x_s[c * T1:(c + 1) * T1, :].astype(F32)
        mu = jnp.mean(xf, axis=1, keepdims=True)
        xc = xf - mu
        var = jnp.mean(xc * xc, axis=1, keepdims=True)
        ln = (xc * jax.lax.rsqrt(var + EPS)).astype(BF16)
        kk = _dot(ln, wk_p[...]).astype(BF16)
        for g in range(G):
            k_s[g, c * T1:(c + 1) * T1, :] = kk[:, 128 * g:128 * (g + 1)]
        qv = _dot_nt(wqv_t[...], ln)
        qt_s[0:D, c * T1:(c + 1) * T1] = (qv[0:D] * QSCALE).astype(BF16)
        vt = jnp.where(ones_row, 1.0, qv[D:])
        vt_s[:, c * T1:(c + 1) * T1] = vt.astype(BF16)

    wo_copy.wait()
    wof = wo_s[...].astype(F32)
    for h in range(H):
        rep_s[HP * h:HP * h + DH, :] = wof[DH * h:DH * (h + 1), :]
    wo_t[...] = rep_s[...].T.astype(BF16)

    nq = S // QT
    nk = S // KC
    qrow = jax.lax.broadcasted_iota(jnp.int32, (128, QT), 0)

    def attn_body(i, carry):
        g = i % G
        q0 = pl.multiple_of((i // G) * QT, QT)
        r0 = pl.multiple_of(g * GW, 16)
        qg = qt_s[pl.ds(r0, 128), pl.ds(q0, QT)]
        qms = [jnp.where((qrow >= DH * j) & (qrow < DH * (j + 1)), qg,
                         jnp.zeros_like(qg)) for j in range(4)]
        units = [(j, c) for j in range(4) for c in range(nk)]

        def qk(u):
            j, c = u
            return _dot(k_s[g, c * KC:(c + 1) * KC, :], qms[j])

        s_next = qk(units[0])
        m = None
        o = None
        for idx, (j, c) in enumerate(units):
            s = s_next
            if idx + 1 < len(units):
                s_next = qk(units[idx + 1])
            v0 = pl.multiple_of((g * 4 + j) * HP, HP)
            mc = jnp.max(s, axis=0, keepdims=True)
            m_new = mc if c == 0 else jnp.maximum(m, mc)
            p = jnp.exp2(s - m_new).astype(BF16)
            pv = _dot(vt_s[pl.ds(v0, HP), c * KC:(c + 1) * KC], p)
            o = pv if c == 0 else o * jnp.exp2(m - m_new) + pv
            m = m_new
            if c == nk - 1:
                on = o * (1.0 / o[DH:DH + 1, :])
                ot_s[pl.ds(v0, HP), pl.ds(q0, QT)] = on.astype(BF16)
        return carry

    jax.lax.fori_loop(0, nq * G, attn_body, 0)

    for t in range(S // T3):
        sl = slice(t * T3, (t + 1) * T3)
        attn_t = _dot(wo_t[...], ot_s[:, sl])
        ht = x_s[sl, :].astype(F32).T + attn_t
        ht_s[:, sl] = ht
        mu = jnp.mean(ht, axis=0, keepdims=True)
        hc = ht - mu
        var = jnp.mean(hc * hc, axis=0, keepdims=True)
        ln2_s[:, sl] = (hc * jax.lax.rsqrt(var + EPS)).astype(BF16)

    w1_copy.wait()
    b1_copy.wait()
    for f in range(F // FT):
        sl = slice(f * FT, (f + 1) * FT)
        u = _dot(ln2_s[...], w1_s[:, sl]) + b1_s[:, sl].astype(F32)
        g_s[:, sl] = _gelu_tanh(u).astype(BF16)

    w2_copy.wait()
    b2_copy.wait()
    n5 = S // T5

    def out_copy(t):
        return pltpu.make_async_copy(out_s.at[pl.ds(t * T5, T5)],
                                     out_hbm.at[pl.ds(t * T5, T5)], out_sems.at[t])

    for t in range(n5):
        sl = slice(t * T5, (t + 1) * T5)
        y = _dot(g_s[...], w2_s[:, sl]) + b2_s[:, sl].astype(F32)
        ot = ht_s[:, sl] + y
        out_s[sl, :] = ot.T.astype(BF16)
        out_copy(t).start()
    for t in range(n5):
        out_copy(t).wait()


@jax.jit
def pallas_sequential_preLN__mha_block__mixer_token_mlp__prompt_kernel(
    A_x: jax.Array,
    A_wqkv: jax.Array,
    A_wo: jax.Array,
    B_x: jax.Array,
    B_w1: jax.Array,
    B_b1: jax.Array,
    B_w2: jax.Array,
    B_b2: jax.Array,
):
    del B_x
    x = A_x.reshape(S, D)
    b1 = B_b1.reshape(1, F)
    b2 = B_b2.reshape(1, S)

    n1 = S // T1
    n5 = S // T5
    any_spec = pl.BlockSpec(memory_space=pl.ANY)
    scratch = [
        pltpu.VMEM((S, D), BF16),
        pltpu.VMEM((D, 3 * D), BF16),
        pltpu.VMEM((D, D), BF16),
        pltpu.VMEM((S, F), BF16),
        pltpu.VMEM((1, F), BF16),
        pltpu.VMEM((F, S), BF16),
        pltpu.VMEM((1, S), BF16),
        pltpu.VMEM((D, G * 128), BF16),
        pltpu.VMEM((D + H * HP, D), BF16),
        pltpu.VMEM((D, H * HP), BF16),
        pltpu.VMEM((H * HP, D), F32),
        pltpu.VMEM((G, S, 128), BF16),
        pltpu.VMEM((H * HP, S), BF16),
        pltpu.VMEM((H * HP, S), BF16),
        pltpu.VMEM((H * HP, S), BF16),
        pltpu.VMEM((D, S), F32),
        pltpu.VMEM((D, S), BF16),
        pltpu.VMEM((D, F), BF16),
        pltpu.VMEM((S, D), BF16),
        pltpu.SemaphoreType.DMA((n1 + 6,)),
        pltpu.SemaphoreType.DMA((n5,)),
    ]
    out = pl.pallas_call(
        _kernel,
        out_shape=jax.ShapeDtypeStruct((S, D), BF16),
        in_specs=[any_spec] * 7,
        out_specs=any_spec,
        scratch_shapes=scratch,
        compiler_params=pltpu.CompilerParams(vmem_limit_bytes=100 * 1024 * 1024),
    )(x, A_wqkv, A_wo, B_w1, b1, B_w2, b2)
    return out.reshape(1, S, D)
```

```python
import jax
import jax.numpy as jnp
import jax.experimental.pallas as pl
import jax.experimental.pallas.tpu as pltpu

S = 2048
D = 448
H = 16
DH = 28
F = 1792
HP = 32
G = 4
GW = 4 * DH
EPS = 1e-5
LOG2E = 1.4426950408889634
QSCALE = (DH ** -0.5) * LOG2E

T1 = 512
QT = 512
KC = 128
NK = S // KC
NHT = H * (S // QT)
HPB = 4
DELTA = 2
T3 = 512
FT = 256
T5 = 256
WT_ROWS = 2 * D + H * HP

F32 = jnp.float32
BF16 = jnp.bfloat16


def _dot(a, b):
    return jnp.dot(a, b, preferred_element_type=F32)


def _gelu_tanh(x):
    c = 0.7978845608028654
    return 0.5 * x * (1.0 + jnp.tanh(c * (x + 0.044715 * (x * x * x))))


def _ln_cols(xf):
    mu = jnp.mean(xf, axis=0, keepdims=True)
    xc = xf - mu
    var = jnp.mean(xc * xc, axis=0, keepdims=True)
    return xc * jax.lax.rsqrt(var + EPS)


def _kernel(xt_hbm, wqkv_hbm, wo_hbm, w1_hbm, b1_hbm, w2_hbm, b2_hbm, out_hbm,
            xt_s, wqkv_s, wo_s, w1_s, b1_s, w2_s, b2_s,
            wt_s, wo_t, rep_s,
            k_s, qt_s, vt_s, ot_s, ht_s, ln2_s, g_s, out_s,
            s0, s1, m0, m1, mpart,
            in_sems, out_sems):
    n1 = S // T1

    def x_copy(c):
        return pltpu.make_async_copy(xt_hbm.at[:, pl.ds(c * T1, T1)],
                                     xt_s.at[:, pl.ds(c * T1, T1)], in_sems.at[c])

    wqkv_copy = pltpu.make_async_copy(wqkv_hbm, wqkv_s, in_sems.at[n1])
    wo_copy = pltpu.make_async_copy(wo_hbm, wo_s, in_sems.at[n1 + 1])
    b1_copy = pltpu.make_async_copy(b1_hbm, b1_s, in_sems.at[n1 + 2])
    b2_copy = pltpu.make_async_copy(b2_hbm, b2_s, in_sems.at[n1 + 3])
    w1_copy = pltpu.make_async_copy(w1_hbm, w1_s, in_sems.at[n1 + 4])
    w2_copy = pltpu.make_async_copy(w2_hbm, w2_s, in_sems.at[n1 + 5])

    wqkv_copy.start()
    for c in range(n1):
        x_copy(c).start()
    wo_copy.start()
    b1_copy.start()
    b2_copy.start()

    wqkv_copy.wait()
    w1_copy.start()
    w2_copy.start()

    wt_s[0:2 * D, :] = wqkv_s[:, 0:2 * D].T
    wvt = wqkv_s[:, 2 * D:3 * D].astype(F32).T
    rep_s[...] = jnp.zeros(rep_s.shape, F32)
    for h in range(H):
        rep_s[HP * h:HP * h + DH, :] = wvt[DH * h:DH * (h + 1), :]
    wt_s[2 * D:, :] = rep_s[...].astype(BF16)

    vrow = jax.lax.broadcasted_iota(jnp.int32, (H * HP, T1), 0)
    ones_row = (vrow % HP) == DH

    def ln1(c):
        x_copy(c).wait()
        return _ln_cols(xt_s[:, c * T1:(c + 1) * T1].astype(F32)).astype(BF16)

    ln_next = ln1(0)
    for c in range(n1):
        ln = ln_next
        sl = slice(c * T1, (c + 1) * T1)
        qkv = _dot(wt_s[...], ln)
        if c + 1 < n1:
            ln_next = ln1(c + 1)
        qt_s[:, sl] = (qkv[0:D + 16] * QSCALE).astype(BF16)
        for g in range(G):
            kt = qkv[D + GW * g:D + GW * g + 128].astype(BF16)
            k_s[g, sl, :] = kt.T
        vt_s[:, sl] = jnp.where(ones_row, 1.0, qkv[2 * D:]).astype(BF16)

    wo_copy.wait()
    wof = wo_s[...].astype(F32)
    for h in range(H):
        rep_s[HP * h:HP * h + DH, :] = wof[DH * h:DH * (h + 1), :]
    wo_t[...] = rep_s[...].astype(BF16).T

    qrow = jax.lax.broadcasted_iota(jnp.int32, (128, QT), 0)
    sbuf = (s0, s1)
    mbuf = (m0, m1)

    def decode(ht):
        return ht % H, pl.multiple_of((ht // H) * QT, QT)

    class AState:
        def __init__(self, ht, par, mrun=None):
            h, q0 = decode(ht)
            self.g = h // 4
            lo = (h % 4) * DH
            r0 = pl.multiple_of(self.g * GW, 16)
            qg = qt_s[pl.ds(r0, 128), pl.ds(q0, QT)]
            self.qm = jnp.where((qrow >= lo) & (qrow < lo + DH), qg, jnp.zeros_like(qg))
            self.par = par
            self.mrun = mrun

        def run(self, c):
            s = _dot(k_s[self.g, c * KC:(c + 1) * KC, :], self.qm)
            sbuf[self.par][c * KC:(c + 1) * KC, :] = s
            mc = jnp.max(s.reshape(KC // 8, 8, QT), axis=0)
            self.mrun = mc if self.mrun is None else jnp.maximum(self.mrun, mc)
            if c == NK - 1:
                mbuf[self.par][...] = jnp.max(self.mrun, axis=0, keepdims=True)

    class BState:
        def __init__(self, ht, par):
            h, self.q0 = decode(ht)
            self.v0 = pl.multiple_of(h * HP, HP)
            self.par = par
            self.acc = None
            self.m = None

        def run(self, c):
            if self.m is None:
                self.m = mbuf[self.par][...]
            p = jnp.exp2(sbuf[self.par][c * KC:(c + 1) * KC, :] - self.m).astype(BF16)
            pv = _dot(vt_s[pl.ds(self.v0, HP), c * KC:(c + 1) * KC], p)
            self.acc = pv if self.acc is None else self.acc + pv
            if c == NK - 1:
                on = self.acc * (1.0 / self.acc[DH:DH + 1, :])
                ot_s[pl.ds(self.v0, HP), pl.ds(self.q0, QT)] = on.astype(BF16)

    def tiles(ht0, last):
        astates = {}
        bstates = {}
        for l in range(HPB * NK):
            a = l + NK + DELTA
            rel, c = a // NK, a % NK
            if not (last and rel >= HPB):
                if rel not in astates:
                    mr = mpart[...] if (rel == 1 and DELTA > 0) else None
                    astates[rel] = AState(ht0 + rel, rel % 2, mr)
                astates[rel].run(c)
                if rel == HPB + 1 and c == DELTA - 1:
                    mpart[...] = astates[rel].mrun
            rel = l // NK
            if rel not in bstates:
                bstates[rel] = BState(ht0 + rel, rel % 2)
            bstates[rel].run(l % NK)

    a0 = AState(0, 0)
    for c in range(NK):
        a0.run(c)
    if DELTA > 0:
        a1 = AState(1, 1)
        for c in range(DELTA):
            a1.run(c)
        mpart[...] = a1.mrun

    def attn_body(i, carry):
        tiles(HPB * i, False)
        return carry

    jax.lax.fori_loop(0, NHT // HPB - 1, attn_body, 0)
    tiles(NHT - HPB, True)

    n3 = S // T3

    def outproj(t):
        return _dot(wo_t[...], ot_s[:, t * T3:(t + 1) * T3])

    at_next = outproj(0)
    for t in range(n3):
        sl = slice(t * T3, (t + 1) * T3)
        at = at_next
        if t + 1 < n3:
            at_next = outproj(t + 1)
        ht = xt_s[:, sl].astype(F32) + at
        ht_s[:, sl] = ht
        ln2_s[:, sl] = _ln_cols(ht).astype(BF16)

    w1_copy.wait()
    b1_copy.wait()
    b1 = b1_s[...].astype(F32).reshape(1, F)
    n4 = F // FT

    def mlp1(f):
        return _dot(ln2_s[...], w1_s[:, f * FT:(f + 1) * FT])

    u_next = mlp1(0)
    for f in range(n4):
        sl = slice(f * FT, (f + 1) * FT)
        u = u_next
        if f + 1 < n4:
            u_next = mlp1(f + 1)
        g_s[:, sl] = _gelu_tanh(u + b1[:, sl]).astype(BF16)

    w2_copy.wait()
    b2_copy.wait()
    b2 = b2_s[...].astype(F32).reshape(1, S)
    n5 = S // T5

    def out_copy(t):
        return pltpu.make_async_copy(out_s.at[:, pl.ds(t * T5, T5)],
                                     out_hbm.at[:, pl.ds(t * T5, T5)], out_sems.at[t])

    for t in range(n5):
        sl = slice(t * T5, (t + 1) * T5)
        y = _dot(g_s[...], w2_s[:, sl]) + b2[:, sl]
        out_s[:, sl] = (ht_s[:, sl] + y).astype(BF16)
        out_copy(t).start()
    for t in range(n5):
        out_copy(t).wait()


@jax.jit
def pallas_sequential_preLN__mha_block__mixer_token_mlp__prompt_kernel(
    A_x: jax.Array,
    A_wqkv: jax.Array,
    A_wo: jax.Array,
    B_x: jax.Array,
    B_w1: jax.Array,
    B_b1: jax.Array,
    B_w2: jax.Array,
    B_b2: jax.Array,
):
    del B_x
    xt = jnp.swapaxes(A_x, 1, 2).reshape(D, S)

    n1 = S // T1
    n5 = S // T5
    any_spec = pl.BlockSpec(memory_space=pl.ANY)
    scratch = [
        pltpu.VMEM((D, S), BF16),
        pltpu.VMEM((D, 3 * D), BF16),
        pltpu.VMEM((D, D), BF16),
        pltpu.VMEM((S, F), BF16),
        pltpu.VMEM((F,), BF16),
        pltpu.VMEM((F, S), BF16),
        pltpu.VMEM((S,), BF16),
        pltpu.VMEM((WT_ROWS, D), BF16),
        pltpu.VMEM((D, H * HP), BF16),
        pltpu.VMEM((H * HP, D), F32),
        pltpu.VMEM((G, S, 128), BF16),
        pltpu.VMEM((D + 16, S), BF16),
        pltpu.VMEM((H * HP, S), BF16),
        pltpu.VMEM((H * HP, S), BF16),
        pltpu.VMEM((D, S), F32),
        pltpu.VMEM((D, S), BF16),
        pltpu.VMEM((D, F), BF16),
        pltpu.VMEM((D, S), BF16),
        pltpu.VMEM((S, QT), F32),
        pltpu.VMEM((S, QT), F32),
        pltpu.VMEM((1, QT), F32),
        pltpu.VMEM((1, QT), F32),
        pltpu.VMEM((8, QT), F32),
        pltpu.SemaphoreType.DMA((n1 + 6,)),
        pltpu.SemaphoreType.DMA((n5,)),
    ]
    out_t = pl.pallas_call(
        _kernel,
        out_shape=jax.ShapeDtypeStruct((D, S), BF16),
        in_specs=[any_spec] * 7,
        out_specs=any_spec,
        scratch_shapes=scratch,
        compiler_params=pltpu.CompilerParams(vmem_limit_bytes=100 * 1024 * 1024),
    )(xt, A_wqkv, A_wo, B_w1, B_b1, B_w2, B_b2)
    return jnp.swapaxes(out_t.reshape(1, D, S), 1, 2)
```

```python
import jax
import jax.numpy as jnp
import jax.experimental.pallas as pl
import jax.experimental.pallas.tpu as pltpu

S = 2048
D = 448
H = 16
DH = 28
F = 1792
HP = 32
G = 4
GW = 4 * DH
EPS = 1e-5
LOG2E = 1.4426950408889634
QSCALE = (DH ** -0.5) * LOG2E

T1 = 512
QT = 512
KC = 128
NK = S // KC
NHT = H * (S // QT)
HPB = 12
NIT = 5
DELTA = 3
BA = 1
T3 = 1024
FT = 256
T5 = 128
V0 = 2 * D
WT_ROWS = 3 * D

F32 = jnp.float32
BF16 = jnp.bfloat16


def _dot(a, b):
    return jnp.dot(a, b, preferred_element_type=F32)


def _gelu_tanh(x):
    c = 0.7978845608028654
    return 0.5 * x * (1.0 + jnp.tanh(c * (x + 0.044715 * (x * x * x))))


def _ln_cols(xf):
    mu = jnp.mean(xf, axis=0, keepdims=True)
    xc = xf - mu
    var = jnp.mean(xc * xc, axis=0, keepdims=True)
    return xc * jax.lax.rsqrt(var + EPS)


def _ln_ln_cols(xf):
    mu = jnp.mean(xf, axis=0, keepdims=True)
    xc = xf - mu
    var = jnp.mean(xc * xc, axis=0, keepdims=True)
    r1 = jax.lax.rsqrt(var + EPS)
    r2 = jax.lax.rsqrt(var * (r1 * r1) + EPS)
    return xc * (r1 * r2)


def _kernel(xt_hbm, wqkv_hbm, wo_hbm, w1_hbm, b1_hbm, w2_hbm, b2_hbm, out_hbm,
            xt_s, wqkv_s, wo_s, w1_s, b1_s, w2_s, b2_s,
            wt_s, wo_t, rep_s,
            k_s, qt_s, vt_s, ot_s, ht_s, ln2_s, g_s, out_s,
            s0, s1, m0, m1, mpart,
            in_sems, out_sems):
    n1 = S // T1
    n5 = S // T5

    copies = {}
    for c in range(1, n1):
        copies["x%d" % c] = pltpu.make_async_copy(
            xt_hbm.at[:, pl.ds(c * T1, T1)], xt_s.at[:, pl.ds(c * T1, T1)], in_sems.at[c])
    TH = T1 // 2
    copies["x0a"] = pltpu.make_async_copy(
        xt_hbm.at[:, pl.ds(0, TH)], xt_s.at[:, pl.ds(0, TH)], in_sems.at[0])
    copies["x0b"] = pltpu.make_async_copy(
        xt_hbm.at[:, pl.ds(TH, TH)], xt_s.at[:, pl.ds(TH, TH)], in_sems.at[n1 + 8])
    for i, (name, src, dst) in enumerate([
            ("wA", wqkv_hbm.at[:, 0:512], wqkv_s.at[:, 0:512]),
            ("wB", wqkv_hbm.at[:, 512:2 * D], wqkv_s.at[:, 512:2 * D]),
            ("wC", wqkv_hbm.at[:, 2 * D:3 * D], wqkv_s.at[:, 2 * D:3 * D]),
            ("wo", wo_hbm, wo_s), ("b1", b1_hbm, b1_s),
            ("b2", b2_hbm, b2_s), ("w1", w1_hbm, w1_s), ("w2", w2_hbm, w2_s)]):
        copies[name] = pltpu.make_async_copy(src, dst, in_sems.at[n1 + i])
    for t in range(n5):
        copies["o%d" % t] = pltpu.make_async_copy(
            out_s.at[:, pl.ds(t * T5, T5)], out_hbm.at[:, pl.ds(t * T5, T5)], out_sems.at[t])
    pending = []

    def start(name):
        copies[name].start()
        pending.append(name)

    def wait(name):
        copies[name].wait()
        pending.remove(name)

    for name in ("x0a", "wA", "x0b", "wB", "x1", "wC", "x2", "wo", "x3"):
        start(name)
    start("b1")
    start("b2")

    def ln1(c):
        return _ln_cols(xt_s[:, c * T1:(c + 1) * T1].astype(F32)).astype(BF16)

    def proj_q(c, ln):
        q = _dot(wt_s[0:D, :], ln)
        qt_s[0:D, c * T1:(c + 1) * T1] = (q * QSCALE).astype(BF16)

    def proj_k(c, ln):
        kt = _dot(wt_s[D:V0, :], ln).astype(BF16)
        kt = jnp.concatenate([kt, jnp.zeros((16, T1), BF16)], axis=0)
        for g in range(G):
            k_s[g, c * T1:(c + 1) * T1, :] = kt[GW * g:GW * g + 128].T

    def proj_v(c, ln):
        v = _dot(wt_s[V0:, :], ln)
        tail = jnp.where(jax.lax.broadcasted_iota(jnp.int32, (HP - DH, T1), 0) == 0, 1.0, 0.0)
        for h in range(H):
            blk = jnp.concatenate([v[DH * h:DH * (h + 1)], tail], axis=0)
            vt_s[HP * h:HP * (h + 1), c * T1:(c + 1) * T1] = blk.astype(BF16)

    def ln_cols(lo, hi):
        return _ln_cols(xt_s[:, lo:hi].astype(F32)).astype(BF16)

    def proj_q_cols(lo, hi, ln):
        qt_s[0:D, lo:hi] = (_dot(wt_s[0:D, :], ln) * QSCALE).astype(BF16)

    wait("x0a")
    ln0a = ln_cols(0, TH)
    rep_s[...] = jnp.zeros(rep_s.shape, F32)
    wait("wA")
    wt_s[0:512, :] = wqkv_s[:, 0:512].T
    wait("x0b")
    proj_q_cols(0, TH, ln0a)
    ln0b = ln_cols(TH, T1)
    wait("wB")
    proj_q_cols(TH, T1, ln0b)
    ln0 = jnp.concatenate([ln0a, ln0b], axis=1)
    wt_s[512:2 * D, :] = wqkv_s[:, 512:2 * D].T
    wait("x1")
    proj_k(0, ln0)
    ln1_ = ln1(1)
    proj_q(1, ln1_)
    for name in ("wC", "x2", "x3", "wo"):
        wait(name)
    start("w1")
    start("w2")
    proj_k(1, ln1_)
    wt_s[V0:, :] = wqkv_s[:, 2 * D:3 * D].T
    ln2_ = ln1(2)
    proj_q(2, ln2_)
    proj_k(2, ln2_)
    proj_v(0, ln0)
    ln3_ = ln1(3)
    proj_v(1, ln1_)
    wof = wo_s[...].astype(F32)
    for h in range(H):
        rep_s[HP * h:HP * h + DH, :] = wof[DH * h:DH * (h + 1), :]
    wo_t[...] = rep_s[...].astype(BF16).T
    proj_v(2, ln2_)
    proj_q(3, ln3_)
    proj_k(3, ln3_)
    proj_v(3, ln3_)

    sbuf = (s0, s1)
    mbuf = (m0, m1)

    def decode(ht):
        return ht % H, pl.multiple_of((ht // H) * QT, QT)

    class AState:
        def __init__(self, ht, j, par, mrun=None):
            h, q0 = decode(ht)
            self.g = h // 4
            lo, hi = j * DH, (j + 1) * DH
            a, b = (lo // 16) * 16, -(-hi // 16) * 16
            r0 = pl.multiple_of(self.g * GW + a, 16)
            qg = qt_s[pl.ds(r0, b - a), pl.ds(q0, QT)]
            qrow = jax.lax.broadcasted_iota(jnp.int32, (b - a, QT), 0) + a
            parts = []
            if a > 0:
                parts.append(jnp.zeros((a, QT), BF16))
            parts.append(jnp.where((qrow >= lo) & (qrow < hi), qg, jnp.zeros_like(qg)))
            if b < 128:
                parts.append(jnp.zeros((128 - b, QT), BF16))
            self.qm = jnp.concatenate(parts, axis=0)
            self.par = par
            self.mrun = mrun

        def run(self, c):
            s = _dot(k_s[self.g, c * KC:(c + 1) * KC, :], self.qm)
            sbuf[self.par][c * KC:(c + 1) * KC, :] = s
            mc = jnp.max(s.reshape(KC // 8, 8, QT), axis=0)
            self.mrun = mc if self.mrun is None else jnp.maximum(self.mrun, mc)
            if c == NK - 1:
                mbuf[self.par][...] = jnp.broadcast_to(
                    jnp.max(self.mrun, axis=0, keepdims=True), (8, QT))

    class BState:
        def __init__(self, ht, par):
            h, self.q0 = decode(ht)
            self.v0 = pl.multiple_of(h * HP, HP)
            self.par = par
            self.acc = None
            self.m = None

        def probs(self, c):
            if self.m is None:
                self.m = mbuf[self.par][...]
            sc = sbuf[self.par][c * KC:(c + 1) * KC, :].reshape(KC // 8, 8, QT)
            return jnp.exp2(sc - self.m[None]).reshape(KC, QT).astype(BF16)

        def pv(self, c, p):
            pv = _dot(vt_s[pl.ds(self.v0, HP), c * KC:(c + 1) * KC], p)
            self.acc = pv if self.acc is None else self.acc + pv
            if c == NK - 1:
                on = self.acc * (1.0 / self.acc[DH:DH + 1, :])
                ot_s[pl.ds(self.v0, HP), pl.ds(self.q0, QT)] = on.astype(BF16)

    def tiles(ht0, last, nt=HPB):
        astates = {}
        bstates = {}
        ps = {}
        nslots = nt * NK

        def do_b(u):
            rel = u // NK
            if rel not in bstates:
                bstates[rel] = BState(ht0 + rel, rel % 2)
            ps[u] = bstates[rel].probs(u % NK)

        for u in range(BA):
            do_b(u)
        for l in range(nslots):
            a = l + NK + DELTA
            rel, c = a // NK, a % NK
            if not (last and rel >= nt):
                if rel not in astates:
                    mr = mpart[...] if (rel == 1 and DELTA > 0) else None
                    astates[rel] = AState(ht0 + rel, rel % 4, rel % 2, mr)
                astates[rel].run(c)
                if rel == nt + 1 and c == DELTA - 1:
                    mpart[...] = astates[rel].mrun
            if l + BA < nslots:
                do_b(l + BA)
            bstates[l // NK].pv(l % NK, ps.pop(l))

    a0 = AState(0, 0, 0)
    for c in range(NK):
        a0.run(c)
    if DELTA > 0:
        a1 = AState(1, 1, 1)
        for c in range(DELTA):
            a1.run(c)
        mpart[...] = a1.mrun

    def attn_body(i, carry):
        tiles(HPB * i, False)
        return carry

    jax.lax.fori_loop(0, NIT, attn_body, 0)
    tiles(HPB * NIT, True, NHT - HPB * NIT)

    wait("b1")
    n3 = S // T3

    def outproj(t):
        return _dot(wo_t[...], ot_s[:, t * T3:(t + 1) * T3])

    at_next = outproj(0)
    for t in range(n3):
        sl = slice(t * T3, (t + 1) * T3)
        at = at_next
        if t + 1 < n3:
            at_next = outproj(t + 1)
        ht = xt_s[:, sl].astype(F32) + at
        ht_s[:, sl] = ht
        ln2_s[:, sl] = _ln_ln_cols(ht).astype(BF16)

    wait("w1")
    b1 = b1_s[...].astype(F32).reshape(1, F)
    n4 = F // FT

    def mlp1(f):
        return _dot(ln2_s[...], w1_s[:, f * FT:(f + 1) * FT])

    u_next = mlp1(0)
    for f in range(n4):
        sl = slice(f * FT, (f + 1) * FT)
        u = u_next
        if f + 1 < n4:
            u_next = mlp1(f + 1)
        g_s[:, sl] = _gelu_tanh(u + b1[:, sl]).astype(BF16)

    wait("w2")
    wait("b2")
    b2 = b2_s[...].astype(F32).reshape(1, S)

    for t in range(n5):
        sl = slice(t * T5, (t + 1) * T5)
        y = _dot(g_s[...], w2_s[:, sl]) + b2[:, sl]
        out_s[:, sl] = (ht_s[:, sl] + y).astype(BF16)
        start("o%d" % t)
    for t in range(n5):
        wait("o%d" % t)
    assert not pending


@jax.jit
def pallas_sequential_preLN__mha_block__mixer_token_mlp__prompt_kernel(
    A_x: jax.Array,
    A_wqkv: jax.Array,
    A_wo: jax.Array,
    B_x: jax.Array,
    B_w1: jax.Array,
    B_b1: jax.Array,
    B_w2: jax.Array,
    B_b2: jax.Array,
):
    del B_x
    xt = jnp.swapaxes(A_x, 1, 2).reshape(D, S)

    n1 = S // T1
    n5 = S // T5
    any_spec = pl.BlockSpec(memory_space=pl.ANY)
    scratch = [
        pltpu.VMEM((D, S), BF16),
        pltpu.VMEM((D, 3 * D), BF16),
        pltpu.VMEM((D, D), BF16),
        pltpu.VMEM((S, F), BF16),
        pltpu.VMEM((F,), BF16),
        pltpu.VMEM((F, S), BF16),
        pltpu.VMEM((S,), BF16),
        pltpu.VMEM((WT_ROWS, D), BF16),
        pltpu.VMEM((D, H * HP), BF16),
        pltpu.VMEM((H * HP, D), F32),
        pltpu.VMEM((G, S, 128), BF16),
        pltpu.VMEM((D, S), BF16),
        pltpu.VMEM((H * HP, S), BF16),
        pltpu.VMEM((H * HP, S), BF16),
        pltpu.VMEM((D, S), F32),
        pltpu.VMEM((D, S), BF16),
        pltpu.VMEM((D, F), BF16),
        pltpu.VMEM((D, S), BF16),
        pltpu.VMEM((S, QT), F32),
        pltpu.VMEM((S, QT), F32),
        pltpu.VMEM((8, QT), F32),
        pltpu.VMEM((8, QT), F32),
        pltpu.VMEM((8, QT), F32),
        pltpu.SemaphoreType.DMA((n1 + 9,)),
        pltpu.SemaphoreType.DMA((n5,)),
    ]
    out_t = pl.pallas_call(
        _kernel,
        out_shape=jax.ShapeDtypeStruct((D, S), BF16),
        in_specs=[any_spec] * 7,
        out_specs=any_spec,
        scratch_shapes=scratch,
        compiler_params=pltpu.CompilerParams(vmem_limit_bytes=100 * 1024 * 1024),
    )(xt, A_wqkv, A_wo, B_w1, B_b1, B_w2, B_b2)
    return jnp.swapaxes(out_t.reshape(1, D, S), 1, 2)
```
